```python
import os as _os
_os.environ.setdefault("JAX_PLATFORMS", "cpu")
import jax
import jax.numpy as jnp

def _softmax(x, axis=-1):
    return jax.nn.softmax(x, axis=axis)
def _gelu(x):
    return jax.nn.gelu(x, approximate=True)
def _silu(x):
    return jax.nn.silu(x)
def _sigmoid(x):
    return jax.nn.sigmoid(x)
def _layernorm(x, axis=-1, eps=1e-5):
    m = jnp.mean(x, axis=axis, keepdims=True)
    v = jnp.var(x, axis=axis, keepdims=True)
    return (x - m) / jnp.sqrt(v + eps)
def _scatter_add(tgt, idx, src, axis=0):
    return tgt.at[idx].add(src)
def _segment_sum(src, seg, n):
    return jax.ops.segment_sum(src, seg, n)
class _Rng:
    def __init__(self, key):
        self._k = key
    def _next(self):
        self._k, sub = jax.random.split(self._k)
        return sub
    def normal(self, shape):
        return jax.random.normal(self._next(), shape, dtype=jnp.bfloat16)
    def randint(self, lo, hi, shape):
        return jax.random.randint(self._next(), shape, lo, hi, dtype=jnp.int32)
    def uniform(self, shape, lo=0.0, hi=1.0):
        return jax.random.uniform(self._next(), shape, jnp.bfloat16, lo, hi)
    def permutation(self, n):
        return jax.random.permutation(self._next(), n)


kernel_name = 'concat_heads__gqa_block_cached__gqa_block_cached__near_ridge'

def setup_inputs():
    _rng = _Rng(jax.random.key(int.from_bytes(__import__("os").urandom(4), "little")))
    _w = (lambda a: (lambda t: t.astype(jnp.bfloat16) if jnp.issubdtype(t.dtype, jnp.floating) else t)(jnp.asarray(a)))
    def _A_setup():
        B, Sq, D = 8, 128, 576
        Hq, Hkv, Sk, Dh = 32, 16, 512, 128
        assert Hq % Hkv == 0, (Hq, Hkv)
        return {
            "x": _w((lambda *s: _rng.normal(s) * 0.8)(B, Sq, D)),
            "k_cache": _w((lambda *s: _rng.normal(s) * 0.8)(B, Hkv, Sk, Dh)),
            "v_cache": _w((lambda *s: _rng.normal(s) * 0.05)(B, Hkv, Sk, Dh)),
            "wq": _w((lambda *s: _rng.normal(s) * 0.8)(D, Hq * Dh) * (D ** -0.5)),
            "wo": _w((lambda *s: _rng.normal(s) * 0.05)(Hq * Dh, D) * ((Hq * Dh) ** -0.5)),
        }
    _A_in = _A_setup()

    def _B_setup():
        B, Sq, D = 8, 128, 576
        Hq, Hkv, Sk, Dh = 32, 16, 512, 128
        assert Hq % Hkv == 0, (Hq, Hkv)
        return {
            "x": _w((lambda *s: _rng.normal(s) * 0.8)(B, Sq, D)),
            "k_cache": _w((lambda *s: _rng.normal(s) * 0.8)(B, Hkv, Sk, Dh)),
            "v_cache": _w((lambda *s: _rng.normal(s) * 0.05)(B, Hkv, Sk, Dh)),
            "wq": _w((lambda *s: _rng.normal(s) * 0.8)(D, Hq * Dh) * (D ** -0.5)),
            "wo": _w((lambda *s: _rng.normal(s) * 0.05)(Hq * Dh, D) * ((Hq * Dh) ** -0.5)),
        }
    _B_in = _B_setup()

    return {
        "A_x": _A_in["x"],
        "A_k_cache": _A_in["k_cache"],
        "A_v_cache": _A_in["v_cache"],
        "A_wq": _A_in["wq"],
        "A_wo": _A_in["wo"],
        "B_x": _B_in["x"],
        "B_k_cache": _B_in["k_cache"],
        "B_v_cache": _B_in["v_cache"],
        "B_wq": _B_in["wq"],
        "B_wo": _B_in["wo"],
    }

def reference(A_x, A_k_cache, A_v_cache, A_wq, A_wo, B_x, B_k_cache, B_v_cache, B_wq, B_wo):
    def _A_ref(x, k_cache, v_cache, wq, wo):
        B, Sq, D = x.shape
        Hq, Dh = 32, 128
        Hkv = k_cache.shape[1]
        rep = Hq // Hkv
        q = (lambda x, *d: x.transpose(*d))((x @ wq).reshape(B, Sq, Hq, Dh), 0, 2, 1, 3)
        k = jnp.repeat(k_cache, rep, axis=1)
        v = jnp.repeat(v_cache, rep, axis=1)
        scores = jnp.einsum("bhqd,bhkd->bhqk", q, k) * (Dh ** -0.5)
        p = _softmax(scores, axis=-1)
        o = jnp.einsum("bhqk,bhkd->bhqd", p, v)
        return (lambda x, *d: x.transpose(*d))(o, 0, 2, 1, 3).reshape(B, Sq, Hq * Dh) @ wo

    def _B_ref(x, k_cache, v_cache, wq, wo):
        B, Sq, D = x.shape
        Hq, Dh = 32, 128
        Hkv = k_cache.shape[1]
        rep = Hq // Hkv
        q = (lambda x, *d: x.transpose(*d))((x @ wq).reshape(B, Sq, Hq, Dh), 0, 2, 1, 3)
        k = jnp.repeat(k_cache, rep, axis=1)
        v = jnp.repeat(v_cache, rep, axis=1)
        scores = jnp.einsum("bhqd,bhkd->bhqk", q, k) * (Dh ** -0.5)
        p = _softmax(scores, axis=-1)
        o = jnp.einsum("bhqk,bhkd->bhqd", p, v)
        return (lambda x, *d: x.transpose(*d))(o, 0, 2, 1, 3).reshape(B, Sq, Hq * Dh) @ wo

    a = _A_ref(A_x, A_k_cache, A_v_cache, A_wq, A_wo)
    b = _B_ref(B_x, B_k_cache, B_v_cache, B_wq, B_wo)
    return jnp.concatenate([a, b], axis=-1)
```

```python
import functools, math
import jax, jax.numpy as jnp
from jax import lax
from jax.experimental import pallas as pl
from jax.experimental.pallas import tpu as pltpu

B, SQ, D = 8, 128, 576
HQ, HKV, SK, DH = 32, 16, 512, 128
REP = HQ // HKV
M = B * SQ
QW = REP * DH
QSCALE = (DH ** -0.5) * math.log2(math.e)
NT = (((1,), (1,)), ((), ()))
F32 = jnp.float32
BF16 = jnp.bfloat16


def kernel(ax, ak, av, awq, awo, bx, bk, bv, bwq, bwo, out_hbm,
           xt_buf, x_scr, k_buf, v_buf, wq_buf, wo_buf, q_scr, o_scr, acc, out_stage,
           sem_in, sem_x, sem_out, *, nsteps, qsplit, osplit, unroll, xch, skew, pf_pos):
    X = (ax, bx); K = (ak, bk); V = (av, bv); WQ = (awq, bwq); WO = (awo, bwo)
    XB = B // xch

    def copies(j, slot):
        col = pl.multiple_of(j * QW, QW)
        c = {}
        for br in range(2):
            c["wq", br] = pltpu.make_async_copy(WQ[br].at[:, pl.ds(col, QW)], wq_buf.at[slot, br], sem_in.at[slot, 0, br])
            c["k", br] = pltpu.make_async_copy(K[br].at[:, j], k_buf.at[slot, br], sem_in.at[slot, 1, br])
            c["v", br] = pltpu.make_async_copy(V[br].at[:, j], v_buf.at[slot, br], sem_in.at[slot, 2, br])
            c["wo", br] = pltpu.make_async_copy(WO[br].at[:, pl.ds(col, QW)], wo_buf.at[slot, br], sem_in.at[slot, 3, br])
        return c

    ORDER = [("wq", 0), ("wq", 1), ("k", 0), ("v", 0), ("k", 1), ("v", 1), ("wo", 0), ("wo", 1)]

    def start_all(j, slot):
        c = copies(j, slot)
        for key in ORDER:
            c[key].start()

    def xcopy(br, c):
        return pltpu.make_async_copy(X[br].at[pl.ds(c * XB, XB)], xt_buf.at[br, pl.ds(c * XB, XB)], sem_x.at[br, c])

    def xpose(br, b0, b1):
        for b in range(b0, b1):
            x_scr[br, b * SQ:(b + 1) * SQ, :] = xt_buf[br, b].T

    def qproj(br, slot, b0, b1):
        rows = (b1 - b0) * SQ
        q = jnp.dot(x_scr[br, b0 * SQ:b1 * SQ, :], wq_buf[slot, br], preferred_element_type=F32)
        q = (q * QSCALE).astype(BF16)
        for bb in range(b1 - b0):
            for h in range(REP):
                q_scr[br, b0 + bb, h * SQ:(h + 1) * SQ, :] = q[bb * SQ:(bb + 1) * SQ, h * DH:(h + 1) * DH]

    def qk(br, slot, b):
        return lax.dot_general(q_scr[br, b], k_buf[slot, br, b], NT, preferred_element_type=F32)

    def softmax_pv(br, slot, b, s):
        m = jnp.max(s, axis=-1, keepdims=True)
        p = jnp.exp2(s - m)
        l = jnp.sum(p, axis=-1, keepdims=True)
        o = jnp.dot(p.astype(BF16), v_buf[slot, br, b], preferred_element_type=F32)
        r = pl.reciprocal(l, approx=True)
        r = r * (2.0 - l * r)
        o = (o * r).astype(BF16)
        for h in range(REP):
            o_scr[br, b * SQ:(b + 1) * SQ, h * DH:(h + 1) * DH] = o[h * SQ:(h + 1) * SQ]

    def attention(slot, items):
        if skew:
            s = qk(*items[0][:1], slot, items[0][1])
            for i, (br, b) in enumerate(items):
                s_next = qk(items[i + 1][0], slot, items[i + 1][1]) if i + 1 < len(items) else None
                softmax_pv(br, slot, b, s)
                s = s_next
        else:
            for br, b in items:
                softmax_pv(br, slot, b, qk(br, slot, b))

    def oproj(br, slot, first, r0, r1):
        r = lax.dot_general(wo_buf[slot, br], o_scr[br, r0:r1, :], NT, preferred_element_type=F32)
        if first:
            return r
        return acc[br, :, r0:r1] + r

    def step(j, slot, first=False, last=False):
        c = copies(j, slot)
        if not first:
            for key in ORDER:
                c[key].wait()
            if not last and pf_pos == 0:
                start_all(j + 1, 1 - slot)
            qb = B // qsplit
            for br in range(2):
                for ch in range(qsplit):
                    qproj(br, slot, ch * qb, (ch + 1) * qb)
            if not last and pf_pos == 1:
                start_all(j + 1, 1 - slot)
        else:
            xcopy(0, 0).start()
            c["wq", 0].start()
            for ch in range(1, xch):
                xcopy(0, ch).start()
            for ch in range(xch):
                xcopy(0, ch).wait()
                if ch == 0:
                    c["wq", 0].wait()
                    c["wq", 1].start()
                    for cb in range(xch):
                        xcopy(1, cb).start()
                if ch == 1 or xch == 1:
                    for key in ORDER[2:]:
                        c[key].start()
                    if not last:
                        start_all(1, 1)
                xpose(0, ch * XB, (ch + 1) * XB)
                qproj(0, slot, ch * XB, (ch + 1) * XB)
            for cb in range(xch):
                xcopy(1, cb).wait()
            c["wq", 1].wait()
            for ch in range(xch):
                xpose(1, ch * XB, (ch + 1) * XB)
                qproj(1, slot, ch * XB, (ch + 1) * XB)
        if first:
            c["k", 0].wait(); c["v", 0].wait()
            attention(slot, [(0, b) for b in range(B)])
            c["k", 1].wait(); c["v", 1].wait(); c["wo", 0].wait(); c["wo", 1].wait()
            attention(slot, [(1, b) for b in range(B)])
        else:
            attention(slot, [(br, b) for br in range(2) for b in range(B)])
        rows = M // osplit
        for ch in range(osplit):
            r0, r1 = ch * rows, (ch + 1) * rows
            ra = oproj(0, slot, first, r0, r1)
            rb = oproj(1, slot, first, r0, r1)
            if not last:
                acc[0, :, r0:r1] = ra
                acc[1, :, r0:r1] = rb
            else:
                out_stage[r0:r1, :] = jnp.concatenate([ra, rb], axis=0).T.astype(BF16)
                pltpu.make_async_copy(out_stage.at[pl.ds(r0, rows)], out_hbm.at[pl.ds(r0, rows)], sem_out.at[ch]).start()
        if last:
            for ch in range(osplit):
                pltpu.make_async_copy(out_stage.at[pl.ds(ch * rows, rows)], out_hbm.at[pl.ds(ch * rows, rows)], sem_out.at[ch]).wait()

    step(0, 0, first=True, last=(nsteps == 1))
    if nsteps > 2:
        if unroll == 1:
            def body(j, carry):
                step(j, lax.rem(j, 2))
                return carry
            lax.fori_loop(1, nsteps - 1, body, 0)
        else:
            assert (nsteps - 2) % 2 == 0
            def body(i, carry):
                step(2 * i + 1, 1)
                step(2 * i + 2, 0)
                return carry
            lax.fori_loop(0, (nsteps - 2) // 2, body, 0)
    if nsteps > 1:
        step(nsteps - 1, (nsteps - 1) % 2, last=True)


def make(vmem=64, flags=None, nsteps=HKV, qsplit=4, osplit=4, unroll=1, xch=2, skew=True, pf_pos=0):
    def fn(A_x, A_k, A_v, A_wq, A_wo, B_x, B_k, B_v, B_wq, B_wo):
        args = [A_x.transpose(0, 2, 1), A_k, A_v, A_wq, A_wo.T, B_x.transpose(0, 2, 1), B_k, B_v, B_wq, B_wo.T]
        anyspec = pl.BlockSpec(memory_space=pl.ANY)
        out = pl.pallas_call(
            functools.partial(kernel, nsteps=nsteps, qsplit=qsplit, osplit=osplit, unroll=unroll, xch=xch, skew=skew, pf_pos=pf_pos),
            in_specs=[anyspec] * 10,
            out_specs=anyspec,
            out_shape=jax.ShapeDtypeStruct((M, 2 * D), BF16),
            scratch_shapes=[
                pltpu.VMEM((2, B, D, SQ), BF16),
                pltpu.VMEM((2, M, D), BF16),
                pltpu.VMEM((2, 2, B, SK, DH), BF16),
                pltpu.VMEM((2, 2, B, SK, DH), BF16),
                pltpu.VMEM((2, 2, D, QW), BF16),
                pltpu.VMEM((2, 2, D, QW), BF16),
                pltpu.VMEM((2, B, REP * SQ, DH), BF16),
                pltpu.VMEM((2, M, QW), BF16),
                pltpu.VMEM((2, D, M), F32),
                pltpu.VMEM((M, 2 * D), BF16),
                pltpu.SemaphoreType.DMA((2, 4, 2)),
                pltpu.SemaphoreType.DMA((2, xch)),
                pltpu.SemaphoreType.DMA((osplit,)),
            ],
            compiler_params=pltpu.CompilerParams(vmem_limit_bytes=vmem * 1024 * 1024, flags=flags),
        )(*args)
        return out.reshape(B, SQ, 2 * D)
    return fn


@jax.jit
def pallas_concat_heads__gqa_block_cached__gqa_block_cached__near_ridge_kernel(
    A_x: jax.Array,
    A_k_cache: jax.Array,
    A_v_cache: jax.Array,
    A_wq: jax.Array,
    A_wo: jax.Array,
    B_x: jax.Array,
    B_k_cache: jax.Array,
    B_v_cache: jax.Array,
    B_wq: jax.Array,
    B_wo: jax.Array,
):
    return make()(A_x, A_k_cache, A_v_cache, A_wq, A_wo, B_x, B_k_cache, B_v_cache, B_wq, B_wo)
```

```python
import functools, math
import jax, jax.numpy as jnp
from jax import lax
from jax.experimental import pallas as pl
from jax.experimental.pallas import tpu as pltpu

B, SQ, D = 8, 128, 576
HQ, HKV, SK, DH = 32, 16, 512, 128
REP = HQ // HKV
M = B * SQ
QW = REP * DH
QSCALE = (DH ** -0.5) * math.log2(math.e)
NT = (((1,), (1,)), ((), ()))
F32 = jnp.float32
BF16 = jnp.bfloat16


def kernel(ax, ak, av, awq, awo, bx, bk, bv, bwq, bwo, out_hbm,
           xt_buf, x_scr, k_buf, v_buf, wq_buf, wo_buf, q_scr, o_scr, acc, out_stage,
           sem_in, sem_x, sem_out, *, nsteps, qb, ob, order, lsec, xch):
    X = (ax, bx); K = (ak, bk); V = (av, bv); WQ = (awq, bwq); WO = (awo, bwo)
    XB = B // xch

    def cp(kind, br, j, slot):
        col = pl.multiple_of(j * QW, QW)
        if kind == "wq":
            return pltpu.make_async_copy(WQ[br].at[:, pl.ds(col, QW)], wq_buf.at[slot, br], sem_in.at[slot, 0, br])
        if kind == "k":
            return pltpu.make_async_copy(K[br].at[:, j], k_buf.at[slot, br], sem_in.at[slot, 1, br])
        if kind == "v":
            return pltpu.make_async_copy(V[br].at[:, j], v_buf.at[slot, br], sem_in.at[slot, 2, br])
        return pltpu.make_async_copy(WO[br].at[:, pl.ds(col, QW)], wo_buf.at[slot, br], sem_in.at[slot, 3, br])

    KVO = [("k", 0), ("v", 0), ("k", 1), ("v", 1), ("wo", 0), ("wo", 1)]
    WQS = [("wq", 0), ("wq", 1)]

    def xcopy(br, c):
        return pltpu.make_async_copy(X[br].at[pl.ds(c * XB, XB)], xt_buf.at[br, pl.ds(c * XB, XB)], sem_x.at[br, c])

    def out_copy(b0, b1):
        rows = pl.ds(b0 * SQ, (b1 - b0) * SQ)
        return pltpu.make_async_copy(out_stage.at[rows], out_hbm.at[rows], sem_out.at[b0])

    def xpose(br, b0, b1):
        for b in range(b0, b1):
            x_scr[br, b * SQ:(b + 1) * SQ, :] = xt_buf[br, b].T

    def qproj(br, slot, b0, b1):
        for c0 in range(b0, b1, qb):
            q = jnp.dot(x_scr[br, c0 * SQ:(c0 + qb) * SQ, :], wq_buf[slot, br], preferred_element_type=F32)
            q = (q * QSCALE).astype(BF16)
            for bb in range(qb):
                for h in range(REP):
                    q_scr[slot, br, c0 + bb, h * SQ:(h + 1) * SQ, :] = q[bb * SQ:(bb + 1) * SQ, h * DH:(h + 1) * DH]

    def qk(br, slot, b):
        return lax.dot_general(q_scr[slot, br, b], k_buf[slot, br, b], NT, preferred_element_type=F32)

    def softmax_pv(br, slot, b, s):
        m = jnp.max(s, axis=-1, keepdims=True)
        p = jnp.exp2(s - m)
        l = jnp.sum(p, axis=-1, keepdims=True)
        o = jnp.dot(p.astype(BF16), v_buf[slot, br, b], preferred_element_type=F32)
        r = pl.reciprocal(l, approx=True)
        r = r * (2.0 - l * r)
        o = (o * r).astype(BF16)
        for h in range(REP):
            o_scr[br, b * SQ:(b + 1) * SQ, h * DH:(h + 1) * DH] = o[h * SQ:(h + 1) * SQ]

    def oproj(slot, b0, b1, step, last=False):
        for c0 in range(b0, b1, step):
            r0, r1 = c0 * SQ, (c0 + step) * SQ
            res = []
            for br in range(2):
                r = lax.dot_general(wo_buf[slot, br], o_scr[br, r0:r1, :], NT, preferred_element_type=F32)
                res.append(acc[br, :, r0:r1] + r)
            if not last:
                for br in range(2):
                    acc[br, :, r0:r1] = res[br]
            else:
                out_stage[r0:r1, :] = jnp.concatenate(res, axis=0).astype(BF16).T

    def attention(slot, items, after=None):
        after = after or {}
        s = qk(items[0][0], slot, items[0][1])
        for i, (br, b) in enumerate(items):
            s_next = qk(items[i + 1][0], slot, items[i + 1][1]) if i + 1 < len(items) else None
            softmax_pv(br, slot, b, s)
            for f in after.get(i, []):
                f()
            s = s_next

    ALL = [(br, b) for br in range(2) for b in range(B)]

    xcopy(0, 0).start()
    cp("wq", 0, 0, 0).start()
    for ch in range(1, xch):
        xcopy(0, ch).start()
    acc[...] = jnp.zeros_like(acc)
    for ch in range(xch):
        xcopy(0, ch).wait()
        if ch == 0:
            cp("wq", 0, 1, 1).start()
            for cb in range(xch):
                xcopy(1, cb).start()
        if ch == min(1, xch - 1):
            cp("wq", 1, 0, 0).start()
            cp("wq", 1, 1, 1).start()
            for kind, br in KVO:
                cp(kind, br, 0, 0).start()
        xpose(0, ch * XB, (ch + 1) * XB)
        if ch == 0:
            cp("wq", 0, 0, 0).wait()
        qproj(0, 0, ch * XB, (ch + 1) * XB)
    cp("wq", 0, 1, 1).wait()
    qproj(0, 1, 0, B)
    for cb in range(xch):
        xcopy(1, cb).wait()
    cp("wq", 1, 0, 0).wait()
    cp("wq", 1, 1, 1).wait()
    xpose(1, 0, B)
    qproj(1, 0, 0, B)
    qproj(1, 1, 0, B)
    cp("k", 0, 0, 0).wait(); cp("v", 0, 0, 0).wait()
    for kind, br in WQS:
        cp(kind, br, min(2, HKV - 1), 0).start()
    for kind, br in KVO:
        cp(kind, br, 1, 1).start()
    attention(0, ALL[:B])
    for kind, br in KVO[2:]:
        cp(kind, br, 0, 0).wait()
    attention(0, ALL[B:])
    oproj(0, 0, B, ob)

    def body(j, carry):
        slot = lax.rem(j, 2)
        nxt = 1 - slot
        for kind, br in KVO:
            cp(kind, br, j, slot).wait()
        for kind, br in WQS:
            cp(kind, br, j + 1, nxt).wait()
        j2 = jnp.minimum(j + 2, HKV - 1)
        for kind, br in WQS:
            cp(kind, br, j2, slot).start()
        for kind, br in KVO:
            cp(kind, br, j + 1, nxt).start()
        if order == 0:
            qproj(0, nxt, 0, B); qproj(1, nxt, 0, B)
            attention(slot, ALL)
            oproj(slot, 0, B, ob)
        elif order == 1:
            attention(slot, ALL)
            qproj(0, nxt, 0, B); qproj(1, nxt, 0, B)
            oproj(slot, 0, B, ob)
        elif order == 2:
            attention(slot, ALL)
            oproj(slot, 0, B, ob)
            qproj(0, nxt, 0, B); qproj(1, nxt, 0, B)
        elif order == 3:
            after = {2 * i + 1: [functools.partial(qproj, i // 4, nxt, (i % 4) * 2, (i % 4) * 2 + 2)] for i in range(8)}
            attention(slot, ALL, after)
            oproj(slot, 0, B, ob)
        elif order == 4:
            qproj(0, nxt, 0, B)
            attention(slot, ALL)
            oproj(slot, 0, B, ob)
            qproj(1, nxt, 0, B)
        return carry

    lax.fori_loop(1, nsteps - 1, body, 0)

    j = nsteps - 1
    slot = j % 2
    both = lambda b0, b1: [(br, b) for b in range(b0, b1) for br in range(2)]
    if lsec == 0:
        for kind, br in KVO:
            cp(kind, br, j, slot).wait()
        for kind, br in WQS:
            cp(kind, br, j, 1 - slot).wait()
        attention(slot, ALL)
        for b in range(0, B, ob):
            oproj(slot, b, b + ob, ob, last=True)
            out_copy(b, b + ob).start()
        for b in range(0, B, ob):
            out_copy(b, b + ob).wait()
    else:
        secs = lsec
        n = len(secs) - 1
        barriers = [[cp(kind, br, j, slot) for kind, br in KVO[4:]]] + [[cp(kind, br, j, 1 - slot)] for kind, br in WQS]
        pending = []
        for kind, br in KVO[:4]:
            cp(kind, br, j, slot).wait()
        for i in range(n + 1):
            if i >= 1:
                if barriers:
                    grp = barriers.pop(0)
                    if i == n:
                        for g in barriers:
                            grp = grp + g
                        barriers = []
                else:
                    grp = [pending.pop(0)] if len(pending) > 1 else []
                for c in grp:
                    c.wait()
            if i == 0:
                attention(slot, both(secs[0], secs[1]))
            else:
                def fin(i=i):
                    oproj(slot, secs[i - 1], secs[i], 1, True)
                    c = out_copy(secs[i - 1], secs[i])
                    c.start()
                    pending.append(c)
                if i < n:
                    attention(slot, both(secs[i], secs[i + 1]), {0: [fin]})
                else:
                    fin()
        for c in pending:
            c.wait()


def make(vmem=64, flags=None, nsteps=HKV, qb=2, ob=2, order=0, lsec=0, xch=2):
    def fn(A_x, A_k, A_v, A_wq, A_wo, B_x, B_k, B_v, B_wq, B_wo):
        args = [A_x.transpose(0, 2, 1), A_k, A_v, A_wq, A_wo.T, B_x.transpose(0, 2, 1), B_k, B_v, B_wq, B_wo.T]
        anyspec = pl.BlockSpec(memory_space=pl.ANY)
        out = pl.pallas_call(
            functools.partial(kernel, nsteps=nsteps, qb=qb, ob=ob, order=order, lsec=lsec, xch=xch),
            in_specs=[anyspec] * 10,
            out_specs=anyspec,
            out_shape=jax.ShapeDtypeStruct((M, 2 * D), BF16),
            scratch_shapes=[
                pltpu.VMEM((2, B, D, SQ), BF16),
                pltpu.VMEM((2, M, D), BF16),
                pltpu.VMEM((2, 2, B, SK, DH), BF16),
                pltpu.VMEM((2, 2, B, SK, DH), BF16),
                pltpu.VMEM((2, 2, D, QW), BF16),
                pltpu.VMEM((2, 2, D, QW), BF16),
                pltpu.VMEM((2, 2, B, REP * SQ, DH), BF16),
                pltpu.VMEM((2, M, QW), BF16),
                pltpu.VMEM((2, D, M), F32),
                pltpu.VMEM((M, 2 * D), BF16),
                pltpu.SemaphoreType.DMA((2, 4, 2)),
                pltpu.SemaphoreType.DMA((2, xch)),
                pltpu.SemaphoreType.DMA((B,)),
            ],
            compiler_params=pltpu.CompilerParams(vmem_limit_bytes=vmem * 1024 * 1024, flags=flags),
        )(*args)
        return out.reshape(B, SQ, 2 * D)
    return fn


@jax.jit
def pallas_concat_heads__gqa_block_cached__gqa_block_cached__near_ridge_kernel(
    A_x: jax.Array,
    A_k_cache: jax.Array,
    A_v_cache: jax.Array,
    A_wq: jax.Array,
    A_wo: jax.Array,
    B_x: jax.Array,
    B_k_cache: jax.Array,
    B_v_cache: jax.Array,
    B_wq: jax.Array,
    B_wo: jax.Array,
):
    return make(order=3, lsec=(0,3,5,7,8))(A_x, A_k_cache, A_v_cache, A_wq, A_wo, B_x, B_k_cache, B_v_cache, B_wq, B_wo)
```

```python
import functools
import math

import jax
import jax.numpy as jnp
from jax import lax
from jax.experimental import pallas as pl
from jax.experimental.pallas import tpu as pltpu

B, SQ, D = 8, 128, 576
HQ, HKV, SK, DH = 32, 16, 512, 128
REP = HQ // HKV
QW = REP * DH
M = B * SQ
HALF = B // 2
QB = 2
OB = 2
TAIL = (0, 3, 5, 7, 8)
QSCALE = DH ** -0.5 * math.log2(math.e)
NT = (((1,), (1,)), ((), ()))
F32, BF16 = jnp.float32, jnp.bfloat16


def _kernel(ax, ak, av, awq, awo, bx, bk, bv, bwq, bwo, out_hbm,
            xt_buf, x_scr, k_buf, v_buf, wq_buf, wo_buf, q_scr, o_scr, acc, out_stage,
            sem_in, sem_x, sem_out):
    X, K, V, WQ, WO = (ax, bx), (ak, bk), (av, bv), (awq, bwq), (awo, bwo)
    KVO = [("k", 0), ("v", 0), ("k", 1), ("v", 1), ("wo", 0), ("wo", 1)]
    WQS = [("wq", 0), ("wq", 1)]
    ALL = [(br, b) for br in range(2) for b in range(B)]

    def cp(kind, br, j, slot):
        col = pl.ds(pl.multiple_of(j * QW, QW), QW)
        if kind == "wq":
            return pltpu.make_async_copy(WQ[br].at[:, col], wq_buf.at[slot, br], sem_in.at[slot, 0, br])
        if kind == "k":
            return pltpu.make_async_copy(K[br].at[:, j], k_buf.at[slot, br], sem_in.at[slot, 1, br])
        if kind == "v":
            return pltpu.make_async_copy(V[br].at[:, j], v_buf.at[slot, br], sem_in.at[slot, 2, br])
        return pltpu.make_async_copy(WO[br].at[:, col], wo_buf.at[slot, br], sem_in.at[slot, 3, br])

    def xcopy(br, c):
        rows = pl.ds(c * HALF, HALF)
        return pltpu.make_async_copy(X[br].at[rows], xt_buf.at[br, rows], sem_x.at[br, c])

    def out_copy(b0, b1):
        rows = pl.ds(b0 * SQ, (b1 - b0) * SQ)
        return pltpu.make_async_copy(out_stage.at[rows], out_hbm.at[rows], sem_out.at[b0])

    def xpose(br, b0, b1):
        for b in range(b0, b1):
            x_scr[br, b * SQ:(b + 1) * SQ, :] = xt_buf[br, b].T

    def qproj(br, slot, b0, b1):
        for c in range(b0, b1, QB):
            q = jnp.dot(x_scr[br, c * SQ:(c + QB) * SQ, :], wq_buf[slot, br], preferred_element_type=F32)
            q = (q * QSCALE).astype(BF16)
            for i in range(QB):
                for h in range(REP):
                    q_scr[slot, br, c + i, h * SQ:(h + 1) * SQ, :] = q[i * SQ:(i + 1) * SQ, h * DH:(h + 1) * DH]

    def scores(br, slot, b):
        return lax.dot_general(q_scr[slot, br, b], k_buf[slot, br, b], NT, preferred_element_type=F32)

    def softmax_pv(br, slot, b, s):
        p = jnp.exp2(s - jnp.max(s, axis=-1, keepdims=True))
        l = jnp.sum(p, axis=-1, keepdims=True)
        o = jnp.dot(p.astype(BF16), v_buf[slot, br, b], preferred_element_type=F32)
        r = pl.reciprocal(l, approx=True)
        r = r * (2.0 - l * r)
        o = (o * r).astype(BF16)
        for h in range(REP):
            o_scr[br, b * SQ:(b + 1) * SQ, h * DH:(h + 1) * DH] = o[h * SQ:(h + 1) * SQ]

    def oproj(slot, b0, b1, nb, final=False):
        for c in range(b0, b1, nb):
            r0, r1 = c * SQ, (c + nb) * SQ
            res = [acc[br, :, r0:r1] + lax.dot_general(wo_buf[slot, br], o_scr[br, r0:r1, :], NT,
                                                       preferred_element_type=F32)
                   for br in range(2)]
            if final:
                out_stage[r0:r1, :] = jnp.concatenate(res, axis=0).astype(BF16).T
            else:
                for br in range(2):
                    acc[br, :, r0:r1] = res[br]

    def attention(slot, items, after=None):
        s = scores(items[0][0], slot, items[0][1])
        for i, (br, b) in enumerate(items):
            s_next = scores(items[i + 1][0], slot, items[i + 1][1]) if i + 1 < len(items) else None
            softmax_pv(br, slot, b, s)
            if after and i in after:
                after[i]()
            s = s_next

    xcopy(0, 0).start()
    cp("wq", 0, 0, 0).start()
    xcopy(0, 1).start()
    cp("wq", 0, 1, 1).start()
    acc[...] = jnp.zeros_like(acc)
    xcopy(0, 0).wait()
    xcopy(1, 0).start()
    xcopy(1, 1).start()
    xpose(0, 0, HALF)
    cp("wq", 0, 0, 0).wait()
    qproj(0, 0, 0, HALF)
    xcopy(0, 1).wait()
    cp("wq", 0, 1, 1).wait()
    cp("wq", 1, 0, 0).start()
    cp("wq", 1, 1, 1).start()
    for kind, br in KVO:
        cp(kind, br, 0, 0).start()
    qproj(0, 1, 0, HALF)
    xpose(0, HALF, B)
    qproj(0, 0, HALF, B)
    xcopy(1, 0).wait()
    xcopy(1, 1).wait()
    qproj(0, 1, HALF, B)
    xpose(1, 0, B)
    cp("wq", 1, 0, 0).wait()
    cp("wq", 1, 1, 1).wait()
    qproj(1, 0, 0, B)
    qproj(1, 1, 0, B)
    for kind, br in KVO[:2]:
        cp(kind, br, 0, 0).wait()
    for kind, br in WQS:
        cp(kind, br, 2, 0).start()
    for kind, br in KVO:
        cp(kind, br, 1, 1).start()
    attention(0, ALL[:B])
    for kind, br in KVO[2:]:
        cp(kind, br, 0, 0).wait()
    attention(0, ALL[B:])
    oproj(0, 0, B, OB)

    def body(j, carry):
        slot = lax.rem(j, 2)
        nxt = 1 - slot
        for kind, br in KVO:
            cp(kind, br, j, slot).wait()
        for kind, br in WQS:
            cp(kind, br, j + 1, nxt).wait()

        def prefetch():
            for kind, br in KVO:
                cp(kind, br, j + 1, nxt).start()
            for kind, br in WQS:
                cp(kind, br, jnp.minimum(j + 2, HKV - 1), slot).start()

        after = {0: prefetch}
        for i in range(2 * B // QB):
            br, c = divmod(i * QB, B)
            after[2 * i + 1] = functools.partial(qproj, br, nxt, c, c + QB)
        attention(slot, ALL, after)
        oproj(slot, 0, B, OB)
        return carry

    lax.fori_loop(1, HKV - 1, body, 0)

    j, slot = HKV - 1, (HKV - 1) % 2
    group = lambda g: [(br, b) for b in range(TAIL[g], TAIL[g + 1]) for br in range(2)]

    def finish(g):
        oproj(slot, TAIL[g], TAIL[g + 1], 1, final=True)
        out_copy(TAIL[g], TAIL[g + 1]).start()

    for kind, br in KVO[:4]:
        cp(kind, br, j, slot).wait()
    attention(slot, group(0))
    for kind, br in KVO[4:]:
        cp(kind, br, j, slot).wait()
    attention(slot, group(1), {0: functools.partial(finish, 0)})
    cp("wq", 0, j, 1 - slot).wait()
    attention(slot, group(2), {0: functools.partial(finish, 1)})
    cp("wq", 1, j, 1 - slot).wait()
    attention(slot, group(3), {0: functools.partial(finish, 2)})
    out_copy(TAIL[0], TAIL[1]).wait()
    finish(3)
    for g in range(1, 4):
        out_copy(TAIL[g], TAIL[g + 1]).wait()


@jax.jit
def pallas_concat_heads__gqa_block_cached__gqa_block_cached__near_ridge_kernel(
    A_x: jax.Array,
    A_k_cache: jax.Array,
    A_v_cache: jax.Array,
    A_wq: jax.Array,
    A_wo: jax.Array,
    B_x: jax.Array,
    B_k_cache: jax.Array,
    B_v_cache: jax.Array,
    B_wq: jax.Array,
    B_wo: jax.Array,
):
    args = [A_x.transpose(0, 2, 1), A_k_cache, A_v_cache, A_wq, A_wo.T,
            B_x.transpose(0, 2, 1), B_k_cache, B_v_cache, B_wq, B_wo.T]
    hbm = pl.BlockSpec(memory_space=pl.ANY)
    out = pl.pallas_call(
        _kernel,
        in_specs=[hbm] * 10,
        out_specs=hbm,
        out_shape=jax.ShapeDtypeStruct((M, 2 * D), BF16),
        scratch_shapes=[
            pltpu.VMEM((2, B, D, SQ), BF16),
            pltpu.VMEM((2, M, D), BF16),
            pltpu.VMEM((2, 2, B, SK, DH), BF16),
            pltpu.VMEM((2, 2, B, SK, DH), BF16),
            pltpu.VMEM((2, 2, D, QW), BF16),
            pltpu.VMEM((2, 2, D, QW), BF16),
            pltpu.VMEM((2, 2, B, QW, DH), BF16),
            pltpu.VMEM((2, M, QW), BF16),
            pltpu.VMEM((2, D, M), F32),
            pltpu.VMEM((M, 2 * D), BF16),
            pltpu.SemaphoreType.DMA((2, 4, 2)),
            pltpu.SemaphoreType.DMA((2, 2)),
            pltpu.SemaphoreType.DMA((B,)),
        ],
        compiler_params=pltpu.CompilerParams(vmem_limit_bytes=64 * 1024 * 1024, disable_bounds_checks=True),
    )(*args)
    return out.reshape(B, SQ, 2 * D)
```

```python
import functools
import math

import jax
import jax.numpy as jnp
from jax import lax
from jax.experimental import pallas as pl
from jax.experimental.pallas import tpu as pltpu

B, SQ, D = 8, 128, 576
HQ, HKV, SK, DH = 32, 16, 512, 128
REP = HQ // HKV
QW = REP * DH
M = B * SQ
HALF = B // 2
QB = 2
OB = 2
AHEAD = 2
TAIL = (0, 3, 5, 7, 8)
QSCALE = DH ** -0.5 * math.log2(math.e)
NT = (((1,), (1,)), ((), ()))
F32, BF16 = jnp.float32, jnp.bfloat16


def _kernel(ax, ak, av, awq, awo, bx, bk, bv, bwq, bwo, out_hbm,
            xt_buf, x_scr, k_buf, v_buf, wq_buf, wo_buf, q_scr, o_scr, acc, out_stage,
            sem_in, sem_x, sem_out):
    X, K, V, WQ, WO = (ax, bx), (ak, bk), (av, bv), (awq, bwq), (awo, bwo)
    KVO = [("k", 0), ("v", 0), ("k", 1), ("v", 1), ("wo", 0), ("wo", 1)]
    WQS = [("wq", 0), ("wq", 1)]
    ALL = [(br, b) for br in range(2) for b in range(B)]

    def cp(kind, br, j, slot):
        col = pl.ds(pl.multiple_of(j * QW, QW), QW)
        if kind == "wq":
            return pltpu.make_async_copy(WQ[br].at[:, col], wq_buf.at[slot, br], sem_in.at[slot, 0, br])
        if kind == "k":
            return pltpu.make_async_copy(K[br].at[:, j], k_buf.at[slot, br], sem_in.at[slot, 1, br])
        if kind == "v":
            return pltpu.make_async_copy(V[br].at[:, j], v_buf.at[slot, br], sem_in.at[slot, 2, br])
        return pltpu.make_async_copy(WO[br].at[:, col], wo_buf.at[slot, br], sem_in.at[slot, 3, br])

    def xcopy(br, c):
        rows = pl.ds(c * HALF, HALF)
        return pltpu.make_async_copy(X[br].at[rows], xt_buf.at[br, rows], sem_x.at[br, c])

    def out_copy(b0, b1):
        rows = pl.ds(b0 * SQ, (b1 - b0) * SQ)
        return pltpu.make_async_copy(out_stage.at[rows], out_hbm.at[rows], sem_out.at[b0])

    def xpose(br, b0, b1):
        for b in range(b0, b1):
            x_scr[br, b * SQ:(b + 1) * SQ, :] = xt_buf[br, b].T

    def qproj(br, slot, b0, b1):
        for c in range(b0, b1, QB):
            q = jnp.dot(x_scr[br, c * SQ:(c + QB) * SQ, :], wq_buf[slot, br], preferred_element_type=F32)
            q = (q * QSCALE).astype(BF16)
            for i in range(QB):
                for h in range(REP):
                    q_scr[slot, br, c + i, h * SQ:(h + 1) * SQ, :] = q[i * SQ:(i + 1) * SQ, h * DH:(h + 1) * DH]

    def scores(br, slot, b):
        return lax.dot_general(q_scr[slot, br, b], k_buf[slot, br, b], NT, preferred_element_type=F32)

    def softmax_pv(br, slot, b, s):
        p = jnp.exp2(s - jnp.max(s, axis=-1, keepdims=True))
        l = jnp.sum(p, axis=-1, keepdims=True)
        o = jnp.dot(p.astype(BF16), v_buf[slot, br, b], preferred_element_type=F32)
        r = pl.reciprocal(l, approx=True)
        r = r * (2.0 - l * r)
        o = (o * r).astype(BF16)
        for h in range(REP):
            o_scr[br, b * SQ:(b + 1) * SQ, h * DH:(h + 1) * DH] = o[h * SQ:(h + 1) * SQ]

    def oproj(slot, b0, b1, nb, final=False):
        for c in range(b0, b1, nb):
            r0, r1 = c * SQ, (c + nb) * SQ
            res = [acc[br, :, r0:r1] + lax.dot_general(wo_buf[slot, br], o_scr[br, r0:r1, :], NT,
                                                       preferred_element_type=F32)
                   for br in range(2)]
            if final:
                out_stage[r0:r1, :] = jnp.concatenate(res, axis=0).astype(BF16).T
            else:
                for br in range(2):
                    acc[br, :, r0:r1] = res[br]

    def attention(slot, items, after=None):
        pend = [scores(br, slot, b) for br, b in items[:AHEAD]]
        for i, (br, b) in enumerate(items):
            if i + AHEAD < len(items):
                pend.append(scores(items[i + AHEAD][0], slot, items[i + AHEAD][1]))
            softmax_pv(br, slot, b, pend.pop(0))
            if after and i in after:
                after[i]()

    xcopy(0, 0).start()
    cp("wq", 0, 0, 0).start()
    xcopy(0, 1).start()
    cp("wq", 0, 1, 1).start()
    acc[...] = jnp.zeros_like(acc)
    xcopy(0, 0).wait()
    xcopy(1, 0).start()
    xcopy(1, 1).start()
    xpose(0, 0, HALF)
    cp("wq", 0, 0, 0).wait()
    qproj(0, 0, 0, HALF)
    xcopy(0, 1).wait()
    cp("wq", 0, 1, 1).wait()
    cp("wq", 1, 0, 0).start()
    cp("wq", 1, 1, 1).start()
    for kind, br in KVO:
        cp(kind, br, 0, 0).start()
    qproj(0, 1, 0, HALF)
    xpose(0, HALF, B)
    qproj(0, 0, HALF, B)
    xcopy(1, 0).wait()
    xcopy(1, 1).wait()
    qproj(0, 1, HALF, B)
    xpose(1, 0, B)
    cp("wq", 1, 0, 0).wait()
    cp("wq", 1, 1, 1).wait()
    qproj(1, 0, 0, B)
    qproj(1, 1, 0, B)
    for kind, br in KVO[:2]:
        cp(kind, br, 0, 0).wait()
    for kind, br in WQS:
        cp(kind, br, 2, 0).start()
    for kind, br in KVO:
        cp(kind, br, 1, 1).start()
    attention(0, ALL[:B])
    for kind, br in KVO[2:]:
        cp(kind, br, 0, 0).wait()
    attention(0, ALL[B:])
    oproj(0, 0, B, OB)

    def body(j, carry):
        slot = lax.rem(j, 2)
        nxt = 1 - slot
        for kind, br in KVO:
            cp(kind, br, j, slot).wait()
        for kind, br in WQS:
            cp(kind, br, j + 1, nxt).wait()

        def prefetch():
            for kind, br in KVO:
                cp(kind, br, j + 1, nxt).start()
            for kind, br in WQS:
                cp(kind, br, jnp.minimum(j + 2, HKV - 1), slot).start()

        after = {0: prefetch}
        for i in range(2 * B // QB):
            br, c = divmod(i * QB, B)
            after[2 * i + 1] = functools.partial(qproj, br, nxt, c, c + QB)
        attention(slot, ALL, after)
        oproj(slot, 0, B, OB)
        return carry

    lax.fori_loop(1, HKV - 1, body, 0)

    j, slot = HKV - 1, (HKV - 1) % 2
    group = lambda g: [(br, b) for b in range(TAIL[g], TAIL[g + 1]) for br in range(2)]

    def finish(g):
        oproj(slot, TAIL[g], TAIL[g + 1], 1, final=True)
        out_copy(TAIL[g], TAIL[g + 1]).start()

    for kind, br in KVO[:4]:
        cp(kind, br, j, slot).wait()
    attention(slot, group(0))
    for kind, br in KVO[4:]:
        cp(kind, br, j, slot).wait()
    attention(slot, group(1), {0: functools.partial(finish, 0)})
    cp("wq", 0, j, 1 - slot).wait()
    attention(slot, group(2), {0: functools.partial(finish, 1)})
    cp("wq", 1, j, 1 - slot).wait()
    attention(slot, group(3), {0: functools.partial(finish, 2)})
    out_copy(TAIL[0], TAIL[1]).wait()
    finish(3)
    for g in range(1, 4):
        out_copy(TAIL[g], TAIL[g + 1]).wait()


@jax.jit
def pallas_concat_heads__gqa_block_cached__gqa_block_cached__near_ridge_kernel(
    A_x: jax.Array,
    A_k_cache: jax.Array,
    A_v_cache: jax.Array,
    A_wq: jax.Array,
    A_wo: jax.Array,
    B_x: jax.Array,
    B_k_cache: jax.Array,
    B_v_cache: jax.Array,
    B_wq: jax.Array,
    B_wo: jax.Array,
):
    args = [A_x.transpose(0, 2, 1), A_k_cache, A_v_cache, A_wq, A_wo.T,
            B_x.transpose(0, 2, 1), B_k_cache, B_v_cache, B_wq, B_wo.T]
    hbm = pl.BlockSpec(memory_space=pl.ANY)
    out = pl.pallas_call(
        _kernel,
        in_specs=[hbm] * 10,
        out_specs=hbm,
        out_shape=jax.ShapeDtypeStruct((M, 2 * D), BF16),
        scratch_shapes=[
            pltpu.VMEM((2, B, D, SQ), BF16),
            pltpu.VMEM((2, M, D), BF16),
            pltpu.VMEM((2, 2, B, SK, DH), BF16),
            pltpu.VMEM((2, 2, B, SK, DH), BF16),
            pltpu.VMEM((2, 2, D, QW), BF16),
            pltpu.VMEM((2, 2, D, QW), BF16),
            pltpu.VMEM((2, 2, B, QW, DH), BF16),
            pltpu.VMEM((2, M, QW), BF16),
            pltpu.VMEM((2, D, M), F32),
            pltpu.VMEM((M, 2 * D), BF16),
            pltpu.SemaphoreType.DMA((2, 4, 2)),
            pltpu.SemaphoreType.DMA((2, 2)),
            pltpu.SemaphoreType.DMA((B,)),
        ],
        compiler_params=pltpu.CompilerParams(vmem_limit_bytes=64 * 1024 * 1024, disable_bounds_checks=True),
    )(*args)
    return out.reshape(B, SQ, 2 * D)
```
